```python
import os as _os
_os.environ.setdefault("JAX_PLATFORMS", "cpu")
import jax
import jax.numpy as jnp

def _softmax(x, axis=-1):
    return jax.nn.softmax(x, axis=axis)
def _gelu(x):
    return jax.nn.gelu(x, approximate=True)
def _silu(x):
    return jax.nn.silu(x)
def _sigmoid(x):
    return jax.nn.sigmoid(x)
def _layernorm(x, axis=-1, eps=1e-5):
    m = jnp.mean(x, axis=axis, keepdims=True)
    v = jnp.var(x, axis=axis, keepdims=True)
    return (x - m) / jnp.sqrt(v + eps)
def _scatter_add(tgt, idx, src, axis=0):
    return tgt.at[idx].add(src)
def _segment_sum(src, seg, n):
    return jax.ops.segment_sum(src, seg, n)
class _Rng:
    def __init__(self, key):
        self._k = key
    def _next(self):
        self._k, sub = jax.random.split(self._k)
        return sub
    def normal(self, shape):
        return jax.random.normal(self._next(), shape, dtype=jnp.bfloat16)
    def randint(self, lo, hi, shape):
        return jax.random.randint(self._next(), shape, lo, hi, dtype=jnp.int32)
    def uniform(self, shape, lo=0.0, hi=1.0):
        return jax.random.uniform(self._next(), shape, jnp.bfloat16, lo, hi)
    def permutation(self, n):
        return jax.random.permutation(self._next(), n)


kernel_name = 'concat_heads__sliding_local_dilated__compressed_kv_cla__prompt'

def setup_inputs():
    _rng = _Rng(jax.random.key(int.from_bytes(__import__("os").urandom(4), "little")))
    _w = (lambda a: (lambda t: t.astype(jnp.bfloat16) if jnp.issubdtype(t.dtype, jnp.floating) else t)(jnp.asarray(a)))
    def _A_setup():
        B, S, D = 1, 2048, 640
        return {
            "x": _w((lambda *s: _rng.normal(s) * 0.2)(B, S, D)),
            "wqkv": _w((lambda *s: _rng.normal(s) * 0.2)(D, 3 * D)),
            "wo": _w((lambda *s: _rng.normal(s) * 0.05)(D, D)),
        }
    _A_in = _A_setup()

    def _B_setup():
        B, H, Sq, Sk, D, M = 1, 32, 2048, 2048, 128, 640
        Dc = 4 * D
        return {
            "x": _w((lambda *s: _rng.normal(s) * 0.8)(B, Sq, M)),
            "c_kv": _w((lambda *s: _rng.normal(s) * 0.8)(B, Sk, Dc)),
            "w_q": _w((lambda *s: _rng.normal(s) * 1.6)(M, H, D) * (M ** -0.5)),
            "w_uk": _w((lambda *s: _rng.normal(s) * 1.6)(Dc, H, D) * (Dc ** -0.5)),
            "w_uv": _w((lambda *s: _rng.normal(s) * 0.8)(Dc, H, D) * (Dc ** -0.5)),
            "w_o": _w((lambda *s: _rng.normal(s) * 0.8)(H, D, M) * ((H * D) ** -0.5)),
        }
    _B_in = _B_setup()

    return {
        "A_x": _A_in["x"],
        "A_wqkv": _A_in["wqkv"],
        "A_wo": _A_in["wo"],
        "B_x": _B_in["x"],
        "B_c_kv": _B_in["c_kv"],
        "B_w_q": _B_in["w_q"],
        "B_w_uk": _B_in["w_uk"],
        "B_w_uv": _B_in["w_uv"],
        "B_w_o": _B_in["w_o"],
    }

def reference(A_x, A_wqkv, A_wo, B_x, B_c_kv, B_w_q, B_w_uk, B_w_uv, B_w_o):
    def _A_ref(x, wqkv, wo):
        B, S, D = x.shape
        H = 32; Dh = D // H
        W, dil = 8, 2
        qkv = (lambda x, *d: x.transpose(*d))((x @ wqkv).reshape(B, S, 3, H, Dh), 2, 0, 3, 1, 4)
        q, k, v = qkv[0], qkv[1], qkv[2]
        scale = Dh ** -0.5
        pos = jnp.arange(S)
        off = jnp.arange(W) * dil
        idx = pos[:, None] - off[None, :]
        mask = idx >= 0
        idx_c = jnp.where(mask, idx, 0).reshape(-1)
        kg = k[:, :, idx_c, :].reshape(B, H, S, W, Dh)
        vg = v[:, :, idx_c, :].reshape(B, H, S, W, Dh)
        logits = jnp.einsum("bhsd,bhswd->bhsw", q, kg) * scale
        logits = jnp.where(mask[None, None, :, :], logits, -1e9)
        attn = _softmax(logits, axis=-1)
        o = jnp.einsum("bhsw,bhswd->bhsd", attn, vg)
        return (lambda x, *d: x.transpose(*d))(o, 0, 2, 1, 3).reshape(B, S, D) @ wo

    def _B_ref(x, c_kv, w_q, w_uk, w_uv, w_o):
        B, Sq, M = x.shape[0], x.shape[1], x.shape[2]
        Sk = c_kv.shape[1]
        H, D = w_q.shape[1], w_q.shape[2]
        q = jnp.einsum("bqm,mhd->bhqd", x, w_q)
        k = jnp.einsum("bkc,chd->bhkd", c_kv, w_uk)
        v = jnp.einsum("bkc,chd->bhkd", c_kv, w_uv)
        scores = jnp.einsum("bhqd,bhkd->bhqk", q, k) * (D ** -0.5)
        off = Sk - Sq
        qi = jnp.arange(Sq)[:, None]
        kj = jnp.arange(Sk)[None, :]
        cmask = kj <= (qi + off)
        scores = jnp.where(cmask[None, None], scores, -1e9)
        p = _softmax(scores, axis=-1)
        ctx = jnp.einsum("bhqk,bhkd->bhqd", p, v)
        return jnp.einsum("bhqd,hdm->bqm", ctx, w_o)

    a = _A_ref(A_x, A_wqkv, A_wo)
    b = _B_ref(B_x, B_c_kv, B_w_q, B_w_uk, B_w_uv, B_w_o)
    return jnp.concatenate([a, b], axis=-1)
```

```python
import functools
import math

import jax
import jax.numpy as jnp
from jax import lax
import jax.experimental.pallas as pl
import jax.experimental.pallas.tpu as pltpu

F32 = jnp.float32
BF16 = jnp.bfloat16
LOG2E = math.log2(math.e)
MASKED = -1e9 * LOG2E
LANES = 128

A_HEADS = 32
A_WIN = 8
A_DIL = 2
HALO = 16
A_SUB = 16
CHUNK = 512
BQ = 128
AHEAD = 2
LAG = 4

_NT = (((1,), (1,)), ((), ()))


def _dot(a, b):
    return jnp.dot(a, b, preferred_element_type=F32)


def _dot_nt(a, b):
    return lax.dot_general(a, b, _NT, preferred_element_type=F32)


def _recip(l):
    r = pl.reciprocal(l, approx=True)
    r = r * (2.0 - l * r)
    return r * (2.0 - l * r)


def _kernel(ax_hbm, awqkv_hbm, awo_hbm, bx_hbm, bc_hbm, wq_hbm, wuk_hbm, wuv_hbm, wo_hbm,
            out_hbm,
            ax_v, awqkv_v, awo_v, bx_v, bc_v, wq_v, wuk_v, wuv_v, wo_v,
            tr_s, tr2_s, wqkv_t, awo_p, qa_s, ka_s, va_s, qc_s, a_stage, k0_s, v0_s, k1_s, v1_s, b_stage,
            in_sem, out_sem, w_sem):
    S, DA = ax_v.shape
    _, H, D = wq_hbm.shape
    M = wo_v.shape[2]
    dh = DA // A_HEADS
    nv = DA // LANES
    nc = S // CHUNK
    n_pairs = H // 2
    CTX = 3

    pairs = [(awqkv_hbm.at[:, pl.ds(t * DA, DA)], awqkv_v.at[t]) for t in range(3)]
    pairs += [(ax_hbm.at[0, pl.ds(c * CHUNK, CHUNK)], ax_v.at[pl.ds(c * CHUNK, CHUNK)]) for c in range(nc)]
    pairs += [(awo_hbm, awo_v), (bx_hbm.at[0], bx_v), (bc_hbm.at[0], bc_v), (wo_hbm, wo_v)]
    loads = [pltpu.make_async_copy(s, d, in_sem.at[i]) for i, (s, d) in enumerate(pairs)]
    ld_w, ld_x = loads[:3], loads[3:3 + nc]
    ld_awo, ld_bx, ld_bc, ld_wo = loads[3 + nc:]
    ld_w[0].start()
    ld_x[0].start()

    def w_copies(j):
        slot = j % 2
        return [pltpu.make_async_copy(src.bitcast(jnp.uint32).at[:, j, :], dst.at[slot], w_sem.at[3 * slot + i])
                for i, (src, dst) in enumerate(((wq_hbm, wq_v), (wuk_hbm, wuk_v), (wuv_hbm, wuv_v)))]

    def permute_rows(dst, src, base):
        for j in range(nv):
            for d in range(dh):
                dst[base + d * A_HEADS:base + (d + 1) * A_HEADS, j * LANES:(j + 1) * LANES] = (
                    src.at[j][pl.ds(base + d, A_HEADS, stride=dh), :].astype(BF16))

    def prep_w(t):
        for j in range(nv):
            tr_s[j, t * DA:(t + 1) * DA] = awqkv_v[t, j * LANES:(j + 1) * LANES, :].astype(F32).T
        permute_rows(wqkv_t, tr_s, t * DA)

    tr_s[:, 3 * DA:, :] = jnp.zeros((nv, tr_s.shape[1] - 3 * DA, LANES), F32)
    tr2_s[:, DA:, :] = jnp.zeros((nv, tr2_s.shape[1] - DA, LANES), F32)
    ka_s[:, 0:HALO, :] = jnp.zeros((nv, HALO, LANES), F32)
    va_s[:, 0:HALO, :] = jnp.zeros((nv, HALO, LANES), F32)
    a_scale = dh ** -0.5 * LOG2E
    a_rows = S // n_pairs

    def a_proj(ci, t):
        r0 = ci * CHUNK
        y = _dot_nt(ax_v[r0:r0 + CHUNK, :], wqkv_t[t * DA:(t + 1) * DA, :])
        if t == 0:
            qa_s[r0:r0 + CHUNK, :] = y * a_scale
        else:
            for j in range(nv):
                (ka_s, va_s)[t - 1][j, HALO + r0:HALO + r0 + CHUNK, :] = y[:, j * LANES:(j + 1) * LANES]

    def a_window(base, off):
        rows = pl.ds(pl.multiple_of(base + off, A_SUB), A_SUB)
        tap = lambda w: pl.ds(base + (HALO + off - w * A_DIL), A_SUB)
        q = qa_s[rows, :]
        logits = []
        for w in range(A_WIN):
            t = functools.reduce(jnp.add, [q[:, j * LANES:(j + 1) * LANES] * ka_s[j, tap(w), :] for j in range(nv)])
            t = t + pltpu.roll(t, 64, 1)
            t = t + pltpu.roll(t, 32, 1)
            if off < w * A_DIL:
                pos = base + off + lax.broadcasted_iota(jnp.int32, (A_SUB, LANES), 0)
                t = jnp.where(pos >= w * A_DIL, t, MASKED)
            logits.append(t)
        m = functools.reduce(jnp.maximum, logits)
        es = [jnp.exp2(t - m) for t in logits]
        inv = _recip(functools.reduce(jnp.add, es))
        ps = [e * inv for e in es]
        for j in range(nv):
            acc = functools.reduce(jnp.add, [ps[w] * va_s[j, tap(w), :] for w in range(A_WIN)])
            qa_s[rows, j * LANES:(j + 1) * LANES] = acc
        if off + A_SUB == a_rows:
            qc_s[2, rows, :] = acc.astype(BF16)

    ld_w[0].wait()
    for cp in ld_w[1:] + ld_x[1:2]:
        cp.start()
    prep_w(0)
    ld_x[0].wait()
    a_proj(0, 0)
    for cp in ld_w[1:] + ld_x[1:2]:
        cp.wait()
    for cp in ld_x[2:] + [ld_awo]:
        cp.start()
    prep_w(1)
    prep_w(2)
    a_proj(1, 0)
    for t in (1, 2):
        for ci in (0, 1):
            a_proj(ci, t)
    for cp in ld_x[2:] + [ld_awo]:
        cp.wait()
    for cp in [ld_bx, ld_bc] + w_copies(0):
        cp.start()
    for j in range(nv):
        tr2_s[j, 0:DA] = awo_v[:, j * LANES:(j + 1) * LANES].astype(F32)
    permute_rows(awo_p, tr2_s, 0)
    for ci in range(2, nc):
        for t in range(3):
            a_proj(ci, t)

    ld_bx.wait()
    ld_bc.wait()
    ld_wo.start()
    b_scale = D ** -0.5 * LOG2E
    heads = ((qc_s.at[0], k0_s, v0_s), (qc_s.at[1], k1_s, v1_s))
    tri = lax.broadcasted_iota(jnp.int32, (BQ, BQ), 1) <= lax.broadcasted_iota(jnp.int32, (BQ, BQ), 0)

    def head_w(w_u, j, e):
        u = w_u[j % 2]
        u = (u << 16) if e == 0 else (u & jnp.uint32(0xFFFF0000))
        return lax.bitcast_convert_type(u, F32).astype(BF16)

    def scores(e, i):
        q_r, k_r, _ = heads[e]
        return _dot_nt(q_r[i * BQ:(i + 1) * BQ, :], k_r[0:(i + 1) * BQ, :])

    def attend(e, i, s):
        n0 = i * BQ
        parts = [s[:, 0:n0]] if i > 0 else []
        parts.append(jnp.where(tri, s[:, n0:n0 + BQ], MASKED))
        m = functools.reduce(jnp.maximum, [jnp.max(t, axis=1, keepdims=True) for t in parts])
        ps = [jnp.exp2(t - m) for t in parts]
        inv = _recip(functools.reduce(jnp.add, [jnp.sum(t, axis=1, keepdims=True) for t in ps]))
        p = jnp.concatenate([t.astype(BF16) for t in ps], axis=1)
        return _dot(p, heads[e][2][0:n0 + BQ, :]), inv

    def pair_body(j, carry):
        for cp in w_copies(j):
            cp.wait()

        @pl.when(j + 1 < n_pairs)
        def _():
            for cp in w_copies(j + 1):
                cp.start()

        def project(src, w_u, t, scale=None):
            y = _dot(src[...], jnp.concatenate([head_w(w_u, j, 0), head_w(w_u, j, 1)], axis=1))
            if scale is not None:
                y = y * scale
            y = y.astype(BF16)
            heads[0][t][...] = y[:, 0:D]
            heads[1][t][...] = y[:, D:2 * D]

        strips = [(e, i) for i in reversed(range(S // BQ)) for e in range(2)]
        qk = lambda t: scores(*strips[t]) if t < len(strips) else None
        late = []

        def flush(keep):
            while len(late) > keep:
                e, i, o, inv = late.pop(0)
                qc_s[CTX + 2 * j + e, i * BQ:(i + 1) * BQ, :] = (o * inv).astype(BF16)

        project(bx_v, wq_v, 0, b_scale)
        a_base = pl.multiple_of(j * a_rows, a_rows)
        for off in range(0, a_rows, A_SUB):
            a_window(a_base, off)
        project(bc_v, wuk_v, 1)
        pend = [qk(0)]
        project(bc_v, wuv_v, 2)
        pend += [qk(t) for t in range(1, AHEAD)]
        for t, (e, i) in enumerate(strips):
            pend.append(qk(t + AHEAD))
            late.append((e, i, *attend(e, i, pend.pop(0))))
            flush(LAG)
        flush(0)
        return carry

    lax.fori_loop(0, n_pairs, pair_body, 0)

    for ci in range(nc):
        r0 = ci * CHUNK
        a_stage[r0:r0 + CHUNK, :] = _dot(qa_s[r0:r0 + CHUNK, :].astype(BF16), awo_p[...]).astype(BF16)
    st_a = pltpu.make_async_copy(a_stage, out_hbm.at[0, :, pl.ds(0, DA)], out_sem.at[0])
    st_a.start()
    ld_wo.wait()

    def st_b(r0, ci):
        rows = pl.ds(r0, CHUNK)
        return pltpu.make_async_copy(b_stage.at[rows], out_hbm.at[0, rows, pl.ds(DA, M)], out_sem.at[1 + ci])

    def b_out(ci, carry):
        r0 = pl.multiple_of(ci * CHUNK, CHUNK)
        ctx = jnp.concatenate([qc_s[CTX + h, pl.ds(r0, CHUNK), :] for h in range(H)], axis=1)
        b_stage[pl.ds(r0, CHUNK), :] = _dot(ctx, wo_v[...].reshape(H * D, M)).astype(BF16)
        st_b(r0, ci).start()
        return carry

    lax.fori_loop(0, nc, b_out, 0)
    st_a.wait()
    for ci in range(nc):
        st_b(ci * CHUNK, ci).wait()


@jax.jit
def pallas_concat_heads__sliding_local_dilated__compressed_kv_cla__prompt_kernel(
    A_x: jax.Array,
    A_wqkv: jax.Array,
    A_wo: jax.Array,
    B_x: jax.Array,
    B_c_kv: jax.Array,
    B_w_q: jax.Array,
    B_w_uk: jax.Array,
    B_w_uv: jax.Array,
    B_w_o: jax.Array,
):
    _, S, DA = A_x.shape
    MB, H, D = B_w_q.shape
    M = B_w_o.shape[2]
    C = B_c_kv.shape[2]
    assert A_x.shape[0] == B_x.shape[0] == 1 and B_x.shape[1] == B_c_kv.shape[1] == S
    assert D == LANES and DA % LANES == 0 and (S // (H // 2)) % A_SUB == 0
    nv = DA // LANES
    pad = 24
    args = (A_x, A_wqkv, A_wo, B_x, B_c_kv, B_w_q, B_w_uk, B_w_uv, B_w_o)
    vm = pltpu.VMEM
    scratch = [
        vm((S, DA), BF16), vm((3, DA, DA), BF16), vm(A_wo.shape, BF16),
        vm((S, MB), BF16), vm((S, C), BF16),
        vm((2, MB, D), jnp.uint32), vm((2, C, D), jnp.uint32), vm((2, C, D), jnp.uint32),
        vm(B_w_o.shape, BF16),
        vm((nv, 3 * DA + pad, LANES), F32), vm((nv, DA + pad, LANES), F32),
        vm((3 * DA, DA), BF16), vm(A_wo.shape, BF16),
        vm((S, DA), F32), vm((nv, HALO + S, LANES), F32), vm((nv, HALO + S, LANES), F32),
        vm((3 + H, S, D), BF16), vm((S, DA), BF16),
        vm((S, D), BF16), vm((S, D), BF16), vm((S, D), BF16), vm((S, D), BF16),
        vm((S, M), BF16),
        pltpu.SemaphoreType.DMA((7 + S // CHUNK,)), pltpu.SemaphoreType.DMA((1 + S // CHUNK,)),
        pltpu.SemaphoreType.DMA((6,)),
    ]
    return pl.pallas_call(
        _kernel,
        out_shape=jax.ShapeDtypeStruct((1, S, DA + M), BF16),
        in_specs=[pl.BlockSpec(memory_space=pl.ANY)] * len(args),
        out_specs=pl.BlockSpec(memory_space=pl.ANY),
        scratch_shapes=scratch,
        compiler_params=pltpu.CompilerParams(vmem_limit_bytes=110 * 1024 * 1024),
    )(*args)
```

```python
import functools
import math

import jax
import jax.numpy as jnp
from jax import lax
import jax.experimental.pallas as pl
import jax.experimental.pallas.tpu as pltpu

F32 = jnp.float32
BF16 = jnp.bfloat16
LOG2E = math.log2(math.e)
MASKED = -1e9 * LOG2E
LANES = 128

A_HEADS = 32
A_WIN = 8
A_DIL = 2
HALO = 16
A_SUB = 16
CHUNK = 512
BQ = 128
AHEAD = 2
LAG = 4

_NT = (((1,), (1,)), ((), ()))


def _dot(a, b):
    return jnp.dot(a, b, preferred_element_type=F32)


def _dot_nt(a, b):
    return lax.dot_general(a, b, _NT, preferred_element_type=F32)


def _recip(l):
    r = pl.reciprocal(l, approx=True)
    r = r * (2.0 - l * r)
    return r * (2.0 - l * r)


def _kernel(ax_hbm, awqkv_hbm, awo_hbm, bx_hbm, bc_hbm, wq_hbm, wuk_hbm, wuv_hbm, wo_hbm,
            out_hbm,
            ax_v, awqkv_v, awo_v, bx_v, bc_v, wq_v, wuk_v, wuv_v, wo_v,
            tr_s, tr2_s, wqkv_t, awo_p, qa_s, ka_s, va_s, qc_s, a_stage, k0_s, v0_s, k1_s, v1_s, b_stage,
            in_sem, out_sem, w_sem):
    S, DA = ax_v.shape
    _, H, D = wq_hbm.shape
    M = wo_v.shape[2]
    dh = DA // A_HEADS
    nv = DA // LANES
    nc = S // CHUNK
    n_pairs = H // 2
    CTX = 3

    pairs = [(awqkv_hbm.at[:, pl.ds(t * DA, DA)], awqkv_v.at[t]) for t in range(3)]
    pairs += [(ax_hbm.at[0, pl.ds(c * CHUNK, CHUNK)], ax_v.at[pl.ds(c * CHUNK, CHUNK)]) for c in range(nc)]
    pairs += [(awo_hbm, awo_v), (bx_hbm.at[0], bx_v), (bc_hbm.at[0], bc_v), (wo_hbm, wo_v)]
    loads = [pltpu.make_async_copy(s, d, in_sem.at[i]) for i, (s, d) in enumerate(pairs)]
    ld_w, ld_x = loads[:3], loads[3:3 + nc]
    ld_awo, ld_bx, ld_bc, ld_wo = loads[3 + nc:]
    ld_w[0].start()
    ld_x[0].start()

    def w_copies(j):
        slot = j % 2
        return [pltpu.make_async_copy(src.bitcast(jnp.uint32).at[:, j, :], dst.at[slot], w_sem.at[3 * slot + i])
                for i, (src, dst) in enumerate(((wq_hbm, wq_v), (wuk_hbm, wuk_v), (wuv_hbm, wuv_v)))]

    def permute_rows(dst, src, base):
        for j in range(nv):
            for d in range(dh):
                dst[base + d * A_HEADS:base + (d + 1) * A_HEADS, j * LANES:(j + 1) * LANES] = (
                    src.at[j][pl.ds(base + d, A_HEADS, stride=dh), :].astype(BF16))

    def prep_w(t):
        for j in range(nv):
            tr_s[j, t * DA:(t + 1) * DA] = awqkv_v[t, j * LANES:(j + 1) * LANES, :].astype(F32).T
        permute_rows(wqkv_t, tr_s, t * DA)

    tr_s[:, 3 * DA:, :] = jnp.zeros((nv, tr_s.shape[1] - 3 * DA, LANES), F32)
    tr2_s[:, DA:, :] = jnp.zeros((nv, tr2_s.shape[1] - DA, LANES), F32)
    ka_s[:, 0:HALO, :] = jnp.zeros((nv, HALO, LANES), F32)
    va_s[:, 0:HALO, :] = jnp.zeros((nv, HALO, LANES), F32)
    a_scale = dh ** -0.5 * LOG2E
    a_rows = S // n_pairs

    def a_proj(ci, t):
        r0 = ci * CHUNK
        y = _dot_nt(ax_v[r0:r0 + CHUNK, :], wqkv_t[t * DA:(t + 1) * DA, :])
        if t == 0:
            qa_s[r0:r0 + CHUNK, :] = y * a_scale
        else:
            for j in range(nv):
                (ka_s, va_s)[t - 1][j, HALO + r0:HALO + r0 + CHUNK, :] = y[:, j * LANES:(j + 1) * LANES]

    def a_window(base, off):
        rows = pl.ds(pl.multiple_of(base + off, A_SUB), A_SUB)
        tap = lambda w: pl.ds(base + (HALO + off - w * A_DIL), A_SUB)
        q = qa_s[rows, :]
        logits = []
        for w in range(A_WIN):
            t = functools.reduce(jnp.add, [q[:, j * LANES:(j + 1) * LANES] * ka_s[j, tap(w), :] for j in range(nv)])
            t = t + pltpu.roll(t, 64, 1)
            t = t + pltpu.roll(t, 32, 1)
            if off < w * A_DIL:
                pos = base + off + lax.broadcasted_iota(jnp.int32, (A_SUB, LANES), 0)
                t = jnp.where(pos >= w * A_DIL, t, MASKED)
            logits.append(t)
        m = functools.reduce(jnp.maximum, logits)
        es = [jnp.exp2(t - m) for t in logits]
        inv = _recip(functools.reduce(jnp.add, es))
        ps = [e * inv for e in es]
        for j in range(nv):
            acc = functools.reduce(jnp.add, [ps[w] * va_s[j, tap(w), :] for w in range(A_WIN)])
            qa_s[rows, j * LANES:(j + 1) * LANES] = acc
        if off + A_SUB == a_rows:
            qc_s[2, rows, :] = acc.astype(BF16)

    ld_w[0].wait()
    for cp in ld_w[1:] + ld_x[1:2]:
        cp.start()
    prep_w(0)
    ld_x[0].wait()
    a_proj(0, 0)
    for cp in ld_w[1:] + ld_x[1:2]:
        cp.wait()
    for cp in ld_x[2:] + [ld_awo]:
        cp.start()
    prep_w(1)
    prep_w(2)
    a_proj(1, 0)
    for t in (1, 2):
        for ci in (0, 1):
            a_proj(ci, t)
    for cp in ld_x[2:] + [ld_awo]:
        cp.wait()
    for cp in [ld_bx, ld_bc] + w_copies(0):
        cp.start()
    for j in range(nv):
        tr2_s[j, 0:DA] = awo_v[:, j * LANES:(j + 1) * LANES].astype(F32)
    permute_rows(awo_p, tr2_s, 0)
    for t in range(3):
        for ci in range(2, nc):
            a_proj(ci, t)

    ld_bx.wait()
    ld_bc.wait()
    ld_wo.start()
    b_scale = D ** -0.5 * LOG2E
    heads = ((qc_s.at[0], k0_s, v0_s), (qc_s.at[1], k1_s, v1_s))
    tri = lax.broadcasted_iota(jnp.int32, (BQ, BQ), 1) <= lax.broadcasted_iota(jnp.int32, (BQ, BQ), 0)

    def head_w(w_u, j, e):
        u = w_u[j % 2]
        u = (u << 16) if e == 0 else (u & jnp.uint32(0xFFFF0000))
        return lax.bitcast_convert_type(u, F32).astype(BF16)

    def tiles(parts):
        return [t[:, c:c + LANES] for t in parts for c in range(0, t.shape[1], LANES)]

    def scores(e, i):
        q_r, k_r, _ = heads[e]
        return _dot_nt(q_r[i * BQ:(i + 1) * BQ, :], k_r[0:(i + 1) * BQ, :])

    def attend(e, i, s):
        n0 = i * BQ
        parts = [s[:, 0:n0]] if i > 0 else []
        parts.append(jnp.where(tri, s[:, n0:n0 + BQ], MASKED))
        m = jnp.max(functools.reduce(jnp.maximum, tiles(parts)), axis=1, keepdims=True)
        ps = [jnp.exp2(t - m) for t in parts]
        inv = _recip(jnp.sum(functools.reduce(jnp.add, tiles(ps)), axis=1, keepdims=True))
        p = jnp.concatenate([t.astype(BF16) for t in ps], axis=1)
        return _dot(p, heads[e][2][0:n0 + BQ, :]), inv

    def pair_body(j, carry):
        for cp in w_copies(j):
            cp.wait()

        @pl.when(j + 1 < n_pairs)
        def _():
            for cp in w_copies(j + 1):
                cp.start()

        def project(src, w_u, t, scale=None):
            y = _dot(src[...], jnp.concatenate([head_w(w_u, j, 0), head_w(w_u, j, 1)], axis=1))
            if scale is not None:
                y = y * scale
            y = y.astype(BF16)
            heads[0][t][...] = y[:, 0:D]
            heads[1][t][...] = y[:, D:2 * D]

        strips = [(e, i) for e in range(2) for i in reversed(range(S // BQ))]
        qk = lambda t: scores(*strips[t]) if t < len(strips) else None
        late = []

        def flush(keep):
            while len(late) > keep:
                e, i, o, inv = late.pop(0)
                qc_s[CTX + 2 * j + e, i * BQ:(i + 1) * BQ, :] = (o * inv).astype(BF16)

        project(bx_v, wq_v, 0, b_scale)
        a_base = pl.multiple_of(j * a_rows, a_rows)
        for off in range(0, a_rows, A_SUB):
            a_window(a_base, off)
        project(bc_v, wuk_v, 1)
        pend = [qk(0)]
        project(bc_v, wuv_v, 2)
        pend += [qk(t) for t in range(1, AHEAD)]
        for t, (e, i) in enumerate(strips):
            pend.append(qk(t + AHEAD))
            late.append((e, i, *attend(e, i, pend.pop(0))))
            flush(LAG)
        flush(0)
        return carry

    lax.fori_loop(0, n_pairs, pair_body, 0)

    a_stage[...] = _dot(qa_s[...].astype(BF16), awo_p[...]).astype(BF16)
    st_a = pltpu.make_async_copy(a_stage, out_hbm.at[0, :, pl.ds(0, DA)], out_sem.at[0])
    st_a.start()
    ld_wo.wait()

    def st_b(r0, ci):
        rows = pl.ds(r0, CHUNK)
        return pltpu.make_async_copy(b_stage.at[rows], out_hbm.at[0, rows, pl.ds(DA, M)], out_sem.at[1 + ci])

    def b_out(ci, carry):
        r0 = pl.multiple_of(ci * CHUNK, CHUNK)
        ctx = jnp.concatenate([qc_s[CTX + h, pl.ds(r0, CHUNK), :] for h in range(H)], axis=1)
        b_stage[pl.ds(r0, CHUNK), :] = _dot(ctx, wo_v[...].reshape(H * D, M)).astype(BF16)
        st_b(r0, ci).start()
        return carry

    lax.fori_loop(0, nc, b_out, 0)
    st_a.wait()
    for ci in range(nc):
        st_b(ci * CHUNK, ci).wait()


@jax.jit
def pallas_concat_heads__sliding_local_dilated__compressed_kv_cla__prompt_kernel(
    A_x: jax.Array,
    A_wqkv: jax.Array,
    A_wo: jax.Array,
    B_x: jax.Array,
    B_c_kv: jax.Array,
    B_w_q: jax.Array,
    B_w_uk: jax.Array,
    B_w_uv: jax.Array,
    B_w_o: jax.Array,
):
    _, S, DA = A_x.shape
    MB, H, D = B_w_q.shape
    M = B_w_o.shape[2]
    C = B_c_kv.shape[2]
    assert A_x.shape[0] == B_x.shape[0] == 1 and B_x.shape[1] == B_c_kv.shape[1] == S
    assert D == LANES and DA % LANES == 0 and (S // (H // 2)) % A_SUB == 0
    nv = DA // LANES
    pad = 24
    args = (A_x, A_wqkv, A_wo, B_x, B_c_kv, B_w_q, B_w_uk, B_w_uv, B_w_o)
    vm = pltpu.VMEM
    scratch = [
        vm((S, DA), BF16), vm((3, DA, DA), BF16), vm(A_wo.shape, BF16),
        vm((S, MB), BF16), vm((S, C), BF16),
        vm((2, MB, D), jnp.uint32), vm((2, C, D), jnp.uint32), vm((2, C, D), jnp.uint32),
        vm(B_w_o.shape, BF16),
        vm((nv, 3 * DA + pad, LANES), F32), vm((nv, DA + pad, LANES), F32),
        vm((3 * DA, DA), BF16), vm(A_wo.shape, BF16),
        vm((S, DA), F32), vm((nv, HALO + S, LANES), F32), vm((nv, HALO + S, LANES), F32),
        vm((3 + H, S, D), BF16), vm((S, DA), BF16),
        vm((S, D), BF16), vm((S, D), BF16), vm((S, D), BF16), vm((S, D), BF16),
        vm((S, M), BF16),
        pltpu.SemaphoreType.DMA((7 + S // CHUNK,)), pltpu.SemaphoreType.DMA((1 + S // CHUNK,)),
        pltpu.SemaphoreType.DMA((6,)),
    ]
    return pl.pallas_call(
        _kernel,
        out_shape=jax.ShapeDtypeStruct((1, S, DA + M), BF16),
        in_specs=[pl.BlockSpec(memory_space=pl.ANY)] * len(args),
        out_specs=pl.BlockSpec(memory_space=pl.ANY),
        scratch_shapes=scratch,
        compiler_params=pltpu.CompilerParams(vmem_limit_bytes=110 * 1024 * 1024),
    )(*args)
```
